```python
import jax
import jax.numpy as jnp

def _softmax(x, axis=-1):
    return jax.nn.softmax(x, axis=axis)
def _gelu(x):
    return jax.nn.gelu(x, approximate=True)
def _silu(x):
    return jax.nn.silu(x)
def _sigmoid(x):
    return jax.nn.sigmoid(x)
def _layernorm(x, axis=-1, eps=1e-5):
    m = jnp.mean(x, axis=axis, keepdims=True)
    v = jnp.var(x, axis=axis, keepdims=True)
    return (x - m) / jnp.sqrt(v + eps)
def _scatter_add(tgt, idx, src, axis=0):
    return tgt.at[idx].add(src)
def _segment_sum(src, seg, n):
    return jax.ops.segment_sum(src, seg, n)
class _Rng:
    def __init__(self, key):
        self._k = key
    def _next(self):
        self._k, sub = jax.random.split(self._k)
        return sub
    def normal(self, shape):
        return jax.random.normal(self._next(), shape, dtype=jnp.bfloat16)
    def randint(self, lo, hi, shape):
        return jax.random.randint(self._next(), shape, lo, hi, dtype=jnp.int32)
    def uniform(self, shape, lo=0.0, hi=1.0):
        return jax.random.uniform(self._next(), shape, jnp.bfloat16, lo, hi)
    def permutation(self, n):
        return jax.random.permutation(self._next(), n)


kernel_name = 'standalone__detection_seg_fpn_lateral__vision'

def setup_inputs():
    _rng = _Rng(jax.random.key(int.from_bytes(__import__("os").urandom(4), "little")))
    _w = (lambda a: (lambda t: t.astype(jnp.bfloat16) if jnp.issubdtype(t.dtype, jnp.floating) else t)(jnp.asarray(a)))
    H = W = (384 // 2) * 2
    C = 384
    k = 1
    return {
        "c_fine": _w((lambda *s: _rng.normal(s) * 0.05)(1, H, W, C)),
        "p_coarse": _w((lambda *s: _rng.normal(s) * 0.05)(1, H // 2, W // 2, C)),
        "w_lat": _w((lambda *s: _rng.normal(s) * 0.05)(C, C)),
        "w_out": _w((lambda *s: _rng.normal(s) * 0.05)(k, k, C, C)),
    }

def reference(c_fine, p_coarse, w_lat, w_out):
    B, H, W, C = c_fine.shape
    k = 1
    lat = jnp.einsum("bhwc,cd->bhwd", c_fine, w_lat)
    up = jnp.repeat(jnp.repeat(p_coarse, 2, axis=1), 2, axis=2)
    m = lat + up
    pad = k // 2
    mp = jnp.pad(m, ((0, 0), (pad, pad), (pad, pad), (0, 0)))
    o = None
    for di in range(k):
        for dj in range(k):
            t = jnp.einsum("bhwc,cd->bhwd", mp[:, di:di + H, dj:dj + W, :], w_out[di, dj])
            o = t if o is None else o + t
    return o
```

```python
import jax
import jax.numpy as jnp
from jax import lax
import jax.experimental.pallas as pl
import jax.experimental.pallas.tpu as pltpu


def _upsample_rows(q):
    n, c = q.shape
    idx = lax.broadcasted_iota(jnp.int32, (8, c), 0) // 2
    outs = []
    for i in range(n // 8):
        v = q[i * 8:(i + 1) * 8]
        outs.append(jnp.take_along_axis(v, idx, axis=0))
        outs.append(jnp.take_along_axis(v, idx + 4, axis=0))
    return jnp.concatenate(outs, axis=0)


@jax.jit
def pallas_standalone__detection_seg_fpn_lateral__vision_kernel(
    c_fine: jax.Array,
    p_coarse: jax.Array,
    w_lat: jax.Array,
    w_out: jax.Array,
):
    _, H, W, C = c_fine.shape
    th = 4

    def kernel(c_ref, p_ref, wl_ref, wo_ref, o_ref, wc_ref):
        @pl.when(pl.program_id(0) == 0)
        def _():
            wc_ref[...] = jnp.dot(
                wl_ref[...], wo_ref[...], preferred_element_type=jnp.float32
            ).astype(wc_ref.dtype)

        def body(r, _):
            q = jnp.dot(p_ref[r], wo_ref[...], preferred_element_type=jnp.float32)
            up = _upsample_rows(q)
            for k in range(2):
                a = jnp.dot(c_ref[2 * r + k], wc_ref[...], preferred_element_type=jnp.float32)
                o_ref[2 * r + k] = (a + up).astype(o_ref.dtype)

        lax.fori_loop(0, th, body, None)

    return pl.pallas_call(
        kernel,
        grid=(H // (2 * th),),
        in_specs=[
            pl.BlockSpec((None, 2 * th, W, C), lambda i: (0, i, 0, 0)),
            pl.BlockSpec((None, th, W // 2, C), lambda i: (0, i, 0, 0)),
            pl.BlockSpec((C, C), lambda i: (0, 0)),
            pl.BlockSpec((None, None, C, C), lambda i: (0, 0, 0, 0)),
        ],
        out_specs=pl.BlockSpec((None, 2 * th, W, C), lambda i: (0, i, 0, 0)),
        out_shape=jax.ShapeDtypeStruct(c_fine.shape, c_fine.dtype),
        scratch_shapes=[pltpu.VMEM((C, C), w_lat.dtype)],
        compiler_params=pltpu.CompilerParams(
            dimension_semantics=("arbitrary",), vmem_limit_bytes=64 * 2**20
        ),
    )(c_fine, p_coarse, w_lat, w_out)
```

```python
import jax
import jax.numpy as jnp
from jax import lax
import jax.experimental.pallas as pl
import jax.experimental.pallas.tpu as pltpu

G = 8
CW = 64
RG = 2
RSEG = 32
WSEG = 32
P_SLOTS = 12
R_BURST = 30
R_PER = 7
N_READ = 80
W_BURST = 40
W_PER = 8


def _udiv(x, d, bound):
    if isinstance(x, int):
        return x // d
    if d & (d - 1) == 0:
        return x >> (d.bit_length() - 1)
    m = -(-(1 << 16) // d)
    assert all((v * m) >> 16 == v // d for v in range(bound))
    return (x * m) >> 16


def _repeat_rows(q):
    n, c = q.shape
    idx = lax.broadcasted_iota(jnp.int32, (8, c), 0) >> 1
    outs = []
    for i in range(n // 8):
        v = q[i * 8:(i + 1) * 8]
        outs.append(jnp.take_along_axis(v, idx, axis=0))
        outs.append(jnp.take_along_axis(v, idx + 4, axis=0))
    return jnp.concatenate(outs, axis=0)


@jax.jit
def pallas_standalone__detection_seg_fpn_lateral__vision_kernel(
    c_fine: jax.Array,
    p_coarse: jax.Array,
    w_lat: jax.Array,
    w_out: jax.Array,
):
    B, H, W, C = c_fine.shape
    dtype = c_fine.dtype
    assert B == 1 and w_out.shape == (1, 1, C, C)
    assert H % (2 * G) == 0 and W % CW == 0

    S = H // (2 * G)
    ncw = W // CW
    n_chunks = S * ncw
    nq = G // RG
    n_groups = n_chunks * nq
    wps = 2 * W // WSEG
    n_writes = S * wps
    n_issue, rest = divmod(n_groups - R_BURST, R_PER)
    w_tail = n_writes - W_BURST - (n_chunks - N_READ) * W_PER

    assert rest == 0 and n_issue <= N_READ and R_BURST % 2 == 0
    assert W_BURST % 4 == 0 and w_tail >= 0
    assert (R_BURST - 1) // (nq * ncw) < P_SLOTS
    for j in range(n_issue):
        assert (R_BURST + (j + 1) * R_PER - 1) // (nq * ncw) - P_SLOTS < j // ncw
    for j in range(0, N_READ, ncw):
        assert R_BURST + min(j, n_issue) * R_PER >= (j // ncw + 1) * nq * ncw
    assert W_BURST <= (N_READ // ncw) * wps
    for t in range(n_chunks - N_READ):
        assert W_BURST + (t + 1) * W_PER <= ((N_READ + t) // ncw) * wps

    def kernel(c_hbm, p_hbm, wl_hbm, wo_hbm, o_hbm,
               buf, pbuf, wl, wo, wc, rsem, wsem, ksem):
        def slot_of(s):
            return s - _udiv(s, P_SLOTS, S) * P_SLOTS

        def start_reads(first, count):
            n = 0
            for t in range(count):
                u = first + t
                chunk = _udiv(u, nq, n_groups)
                bands = pl.ds((u - chunk * nq) * RG, RG)
                s = _udiv(chunk, ncw, n_chunks)
                wi = chunk - s * ncw
                slot = slot_of(s)
                for x in range(0, CW // 2, RSEG):
                    cols = pl.ds(pl.multiple_of(wi * (CW // 2) + x, RSEG), RSEG)
                    pltpu.make_async_copy(
                        p_hbm.at[bands, s, cols], pbuf.at[slot, bands, cols],
                        rsem.at[1, slot]).start(priority=n % 2)
                    n += 1
                for k in range(2):
                    for x in range(0, CW, RSEG):
                        rows = pl.ds(pl.multiple_of(
                            (2 * s + k) * W + wi * CW + x, RSEG), RSEG)
                        pltpu.make_async_copy(
                            c_hbm.at[bands, rows], buf.at[bands, rows],
                            rsem.at[0, slot]).start(priority=n % 2)
                        n += 1

        def wait_unit(s):
            slot = slot_of(s)
            dst = buf.at[:, pl.ds(pl.multiple_of(s * 2 * W, 2 * W), 2 * W)]
            pltpu.make_async_copy(dst, dst, rsem.at[0, slot]).wait()
            dst = pbuf.at[slot]
            pltpu.make_async_copy(dst, dst, rsem.at[1, slot]).wait()

        def start_writes(first, count):
            for t in range(count):
                rows = pl.ds(pl.multiple_of((first + t) * WSEG, WSEG), WSEG)
                pltpu.make_async_copy(
                    buf.at[:, rows], o_hbm.at[:, rows], wsem.at[0]).start()

        def compute(j, start_dmas):
            s = _udiv(j, ncw, n_chunks)
            wi = j - s * ncw
            cols = pl.ds(pl.multiple_of(wi * (CW // 2), CW // 2), CW // 2)
            rows = [pl.ds(pl.multiple_of((2 * s + k) * W + wi * CW, CW), CW)
                    for k in range(2)]
            p = pbuf[slot_of(s), :, cols, :].reshape(G * CW // 2, C)
            up = _repeat_rows(
                jnp.dot(p, wo[...], preferred_element_type=jnp.float32))
            c = jnp.concatenate(
                [buf[:, r, :].reshape(G * CW, C) for r in rows], axis=0)
            lat = jnp.dot(c, wc[...], preferred_element_type=jnp.float32)
            start_dmas()
            for k, r in enumerate(rows):
                o = lat[k * G * CW:(k + 1) * G * CW] + up
                buf[:, r, :] = o.astype(dtype).reshape(G, CW, C)

        def wait_if_new_unit(j):
            s = _udiv(j, ncw, n_chunks)
            pl.when(j == s * ncw)(lambda: wait_unit(s))

        wl_copy = pltpu.make_async_copy(wl_hbm, wl, ksem.at[0])
        wo_copy = pltpu.make_async_copy(wo_hbm, wo, ksem.at[1])
        wl_copy.start(priority=0)
        wo_copy.start(priority=1)
        early = min(R_BURST // 2, 6)
        lax.fori_loop(0, early, lambda i, _: start_reads(2 * i, 2), None)
        wl_copy.wait()
        wo_copy.wait()
        wc[...] = jnp.dot(
            wl[...], wo[...], preferred_element_type=jnp.float32).astype(dtype)
        lax.fori_loop(early, R_BURST // 2, lambda i, _: start_reads(2 * i, 2), None)

        def read_step(j, _):
            wait_if_new_unit(j)
            compute(j, lambda: start_reads(R_BURST + j * R_PER, R_PER))

        def drain_step(j, _):
            wait_if_new_unit(j)
            compute(j, lambda: None)

        lax.fori_loop(0, n_issue, read_step, None)
        lax.fori_loop(n_issue, N_READ, drain_step, None)
        for s in range(-(-N_READ // ncw), S):
            wait_unit(s)

        def write_step(j, _):
            compute(j, lambda: start_writes(W_BURST + (j - N_READ) * W_PER, W_PER))

        lax.fori_loop(0, W_BURST // 4, lambda i, _: start_writes(4 * i, 4), None)
        lax.fori_loop(N_READ, n_chunks, write_step, None)
        lax.fori_loop(n_writes - w_tail, n_writes,
                      lambda i, _: start_writes(i, 1), None)
        pltpu.make_async_copy(buf, buf, wsem.at[0]).wait()

    out = pl.pallas_call(
        kernel,
        in_specs=[pl.BlockSpec(memory_space=pl.ANY)] * 4,
        out_specs=pl.BlockSpec(memory_space=pl.ANY),
        out_shape=jax.ShapeDtypeStruct((G, S * 2 * W, C), dtype),
        scratch_shapes=[
            pltpu.VMEM((G, S * 2 * W, C), dtype),
            pltpu.VMEM((P_SLOTS, G, W // 2, C), dtype),
            pltpu.VMEM((C, C), dtype),
            pltpu.VMEM((C, C), dtype),
            pltpu.VMEM((C, C), dtype),
            pltpu.SemaphoreType.DMA((2, P_SLOTS)),
            pltpu.SemaphoreType.DMA((1,)),
            pltpu.SemaphoreType.DMA((2,)),
        ],
        compiler_params=pltpu.CompilerParams(
            vmem_limit_bytes=127 * 2**20, disable_bounds_checks=True),
    )(
        c_fine.reshape(G, S * 2 * W, C),
        p_coarse.reshape(G, S, W // 2, C),
        w_lat,
        w_out.reshape(C, C),
    )
    return out.reshape(B, H, W, C)
```

```python
import jax
import jax.numpy as jnp
from jax import lax
import jax.experimental.pallas as pl
import jax.experimental.pallas.tpu as pltpu

G = 8
CW = 64
SEG = 32
RG = 2
WG = 4
P_SLOTS = 12
R_EARLY = 12
R_BURST = 44
R_PER = 7
W_BURST = 16
W_PER = 8
OVERLAP = 64


def _udiv(x, d, bound):
    if isinstance(x, int):
        return x // d
    if d & (d - 1) == 0:
        return x >> (d.bit_length() - 1)
    m = -(-(1 << 16) // d)
    assert all((v * m) >> 16 == v // d for v in range(bound))
    return (x * m) >> 16


def _repeat_rows(q):
    n, c = q.shape
    idx = lax.broadcasted_iota(jnp.int32, (8, c), 0) >> 1
    outs = []
    for i in range(n // 8):
        v = q[i * 8:(i + 1) * 8]
        outs.append(jnp.take_along_axis(v, idx, axis=0))
        outs.append(jnp.take_along_axis(v, idx + 4, axis=0))
    return jnp.concatenate(outs, axis=0)


@jax.jit
def pallas_standalone__detection_seg_fpn_lateral__vision_kernel(
    c_fine: jax.Array,
    p_coarse: jax.Array,
    w_lat: jax.Array,
    w_out: jax.Array,
):
    B, H, W, C = c_fine.shape
    dtype = c_fine.dtype
    assert B == 1 and w_out.shape == (1, 1, C, C)
    assert H % (2 * G) == 0 and W % CW == 0

    n_units = H // (2 * G)
    ncw = W // CW
    n_chunks = n_units * ncw
    spc = 2 * CW // SEG
    spu = spc * ncw
    n_steps = n_units * spu
    n_read, rest = divmod(n_steps - R_BURST, R_PER)
    w_tail = n_steps - W_BURST - (n_chunks - n_read) * W_PER

    assert rest == 0 and G % spc == 0 and W_BURST % 2 == 0 and w_tail >= 0
    assert (R_BURST - 1) // spu < P_SLOTS
    for j in range(n_read):
        assert R_BURST + j * R_PER >= (j // ncw + 1) * spu
        assert (R_BURST + (j + 1) * R_PER - 1) // spu - P_SLOTS < j // ncw
    for j in range(n_read, n_chunks):
        done = (j // ncw) * spu + (j % ncw) * (CW // SEG)
        assert W_BURST + (j - n_read + 1) * W_PER <= done
    assert n_read <= (n_units - 1) * ncw

    def kernel(c_hbm, p_hbm, wl_hbm, wo_hbm, o_hbm,
               buf, pbuf, wl, wo, wc, rsem, wsem, ksem):
        def slot_of(unit):
            return unit - _udiv(unit, P_SLOTS, n_units) * P_SLOTS

        def start_reads(first, count):
            for t in range(count):
                step = first + t
                chunk = _udiv(step, spc, n_steps)
                unit = _udiv(chunk, ncw, n_chunks)
                slot = slot_of(unit)
                cols = pl.ds(pl.multiple_of(
                    (chunk - unit * ncw) * (CW // 2), CW // 2), CW // 2)
                rows = pl.ds(pl.multiple_of(step * SEG, SEG), SEG)
                copies = []
                for g in range(G // spc):
                    band = (step - chunk * spc) * (G // spc) + g
                    copies.append(pltpu.make_async_copy(
                        p_hbm.at[band, unit, cols], pbuf.at[slot, band, cols],
                        rsem.at[1, slot]))
                for g in range(0, G, RG):
                    copies.append(pltpu.make_async_copy(
                        c_hbm.at[pl.ds(g, RG), rows], buf.at[pl.ds(g, RG), rows],
                        rsem.at[0, slot]))
                for n, copy in enumerate(copies):
                    copy.start(priority=n % 2)

        def wait_bytes_of(ref, sem):
            pltpu.make_async_copy(ref, ref, sem).wait()

        def wait_unit(unit):
            slot = slot_of(unit)
            rows = pl.ds(pl.multiple_of(unit * 2 * W, 2 * W), 2 * W)
            wait_bytes_of(buf.at[:, rows], rsem.at[0, slot])
            wait_bytes_of(pbuf.at[slot], rsem.at[1, slot])

        def start_writes(first, count):
            for t in range(count):
                rows = pl.ds(pl.multiple_of((first + t) * SEG, SEG), SEG)
                for n, g in enumerate(range(0, G, WG)):
                    pltpu.make_async_copy(
                        buf.at[pl.ds(g, WG), rows], o_hbm.at[pl.ds(g, WG), rows],
                        wsem.at[0]).start(priority=n % 2)

        def compute(j, start_dmas):
            unit = _udiv(j, ncw, n_chunks)
            wi = j - unit * ncw
            cols = pl.ds(pl.multiple_of(wi * (CW // 2), CW // 2), CW // 2)
            rows = [pl.ds(pl.multiple_of((2 * unit + k) * W + wi * CW, CW), CW)
                    for k in range(2)]
            p = pbuf[slot_of(unit), :, cols, :].reshape(G * CW // 2, C)
            up = _repeat_rows(
                jnp.dot(p, wo[...], preferred_element_type=jnp.float32))
            c = jnp.concatenate(
                [buf[:, r, :].reshape(G * CW, C) for r in rows], axis=0)
            lat = jnp.dot(c, wc[...], preferred_element_type=jnp.float32)
            start_dmas()
            for k, r in enumerate(rows):
                o = lat[k * G * CW:(k + 1) * G * CW] + up
                buf[:, r, :] = o.astype(dtype).reshape(G, CW, C)

        wl_copy = pltpu.make_async_copy(wl_hbm, wl, ksem.at[0])
        wo_copy = pltpu.make_async_copy(wo_hbm, wo, ksem.at[1])
        wl_copy.start(priority=0)
        wo_copy.start(priority=1)
        lax.fori_loop(0, R_EARLY, lambda i, _: start_reads(i, 1), None)
        wl_copy.wait()
        wo_copy.wait()
        wc[...] = jnp.dot(
            wl[...], wo[...], preferred_element_type=jnp.float32).astype(dtype)
        lax.fori_loop(R_EARLY, R_BURST, lambda i, _: start_reads(i, 1), None)

        def read_phase(j, _):
            unit = _udiv(j, ncw, n_chunks)
            pl.when(j == unit * ncw)(lambda: wait_unit(unit))
            compute(j, lambda: start_reads(R_BURST + j * R_PER, R_PER))

        lax.fori_loop(0, n_read, read_phase, None)

        last = n_units - 1
        for unit in range(-(-n_read // ncw), last):
            wait_unit(unit)
        split = n_steps * SEG - OVERLAP
        wait_bytes_of(buf.at[:, last * 2 * W:split], rsem.at[0, slot_of(last)])
        lax.fori_loop(0, W_BURST // 2, lambda i, _: start_writes(2 * i, 2), None)
        wait_bytes_of(buf.at[:, split:], rsem.at[0, slot_of(last)])
        wait_bytes_of(pbuf.at[slot_of(last)], rsem.at[1, slot_of(last)])

        def write_phase(j, _):
            compute(j, lambda: start_writes(W_BURST + (j - n_read) * W_PER, W_PER))

        lax.fori_loop(n_read, n_chunks, write_phase, None)
        lax.fori_loop(n_steps - w_tail, n_steps,
                      lambda i, _: start_writes(i, 1), None)
        wait_bytes_of(buf, wsem.at[0])

    out = pl.pallas_call(
        kernel,
        in_specs=[pl.BlockSpec(memory_space=pl.ANY)] * 4,
        out_specs=pl.BlockSpec(memory_space=pl.ANY),
        out_shape=jax.ShapeDtypeStruct((G, n_units * 2 * W, C), dtype),
        scratch_shapes=[
            pltpu.VMEM((G, n_units * 2 * W, C), dtype),
            pltpu.VMEM((P_SLOTS, G, W // 2, C), dtype),
            pltpu.VMEM((C, C), dtype),
            pltpu.VMEM((C, C), dtype),
            pltpu.VMEM((C, C), dtype),
            pltpu.SemaphoreType.DMA((2, P_SLOTS)),
            pltpu.SemaphoreType.DMA((1,)),
            pltpu.SemaphoreType.DMA((2,)),
        ],
        compiler_params=pltpu.CompilerParams(
            vmem_limit_bytes=127 * 2**20,
            disable_bounds_checks=True,
            disable_semaphore_checks=True,
        ),
    )(
        c_fine.reshape(G, n_units * 2 * W, C),
        p_coarse.reshape(G, n_units, W // 2, C),
        w_lat,
        w_out.reshape(C, C),
    )
    return out.reshape(B, H, W, C)
```

```python
import jax
import jax.numpy as jnp
from jax import lax
import jax.experimental.pallas as pl
import jax.experimental.pallas.tpu as pltpu

G = 8
CW = 64
SEG = 32
RG = 2
WG = 4
P_SLOTS = 12
R_EARLY = 12
R_BURST = 44
R_PER = 7
W_BURST = 16
W_PER = 8
R_TAIL = 2


def _udiv(x, d, bound):
    if isinstance(x, int):
        return x // d
    if d & (d - 1) == 0:
        return x >> (d.bit_length() - 1)
    m = -(-(1 << 16) // d)
    assert all((v * m) >> 16 == v // d for v in range(bound))
    return (x * m) >> 16


def _repeat_rows(q):
    n, c = q.shape
    idx = lax.broadcasted_iota(jnp.int32, (8, c), 0) >> 1
    outs = []
    for i in range(n // 8):
        v = q[i * 8:(i + 1) * 8]
        outs.append(jnp.take_along_axis(v, idx, axis=0))
        outs.append(jnp.take_along_axis(v, idx + 4, axis=0))
    return jnp.concatenate(outs, axis=0)


@jax.jit
def pallas_standalone__detection_seg_fpn_lateral__vision_kernel(
    c_fine: jax.Array,
    p_coarse: jax.Array,
    w_lat: jax.Array,
    w_out: jax.Array,
):
    B, H, W, C = c_fine.shape
    dtype = c_fine.dtype
    assert B == 1 and w_out.shape == (1, 1, C, C)
    assert H % (2 * G) == 0 and W % CW == 0

    n_units = H // (2 * G)
    ncw = W // CW
    n_chunks = n_units * ncw
    spc = 2 * CW // SEG
    spu = spc * ncw
    n_steps = n_units * spu
    n_read, rest = divmod(n_steps - R_BURST, R_PER)
    w_tail = n_steps - W_BURST - (n_chunks - n_read) * W_PER

    assert rest == 0 and G % spc == 0 and W_BURST % 2 == 0 and w_tail >= 0
    assert (R_BURST - 1) // spu < P_SLOTS
    for j in range(n_read):
        assert R_BURST + j * R_PER >= (j // ncw + 1) * spu
        assert (R_BURST + (j + 1) * R_PER - 1) // spu - P_SLOTS < j // ncw
    for j in range(n_read, n_chunks):
        done = (j // ncw) * spu + (j % ncw) * (CW // SEG)
        assert W_BURST + (j - n_read + 1) * W_PER <= done
    assert n_read <= (n_units - 1) * ncw and 0 < R_TAIL < spu

    def kernel(c_hbm, p_hbm, wl_hbm, wo_hbm, o_hbm,
               buf, pbuf, wl, wo, wc, csem, psem, wsem, ksem):
        def slot_of(unit):
            return unit - _udiv(unit, P_SLOTS, n_units) * P_SLOTS

        def start_reads(first, count):
            for t in range(count):
                step = first + t
                chunk = _udiv(step, spc, n_steps)
                unit = _udiv(chunk, ncw, n_chunks)
                slot = slot_of(unit)
                cols = pl.ds(pl.multiple_of(
                    (chunk - unit * ncw) * (CW // 2), CW // 2), CW // 2)
                rows = pl.ds(pl.multiple_of(step * SEG, SEG), SEG)
                c_sem = csem.at[jnp.where(step < n_steps - R_TAIL, slot, P_SLOTS)]
                copies = []
                for g in range(G // spc):
                    band = (step - chunk * spc) * (G // spc) + g
                    copies.append(pltpu.make_async_copy(
                        p_hbm.at[band, unit, cols], pbuf.at[slot, band, cols],
                        psem.at[slot]))
                for g in range(0, G, RG):
                    copies.append(pltpu.make_async_copy(
                        c_hbm.at[pl.ds(g, RG), rows], buf.at[pl.ds(g, RG), rows],
                        c_sem))
                for n, copy in enumerate(copies):
                    copy.start(priority=n % 2)

        def wait_filled(ref, sem):
            pltpu.make_async_copy(ref, ref, sem).wait()

        def wait_unit(unit):
            slot = slot_of(unit)
            rows = pl.ds(pl.multiple_of(unit * 2 * W, 2 * W), 2 * W)
            wait_filled(buf.at[:, rows], csem.at[slot])
            wait_filled(pbuf.at[slot], psem.at[slot])

        def start_writes(first, count):
            for t in range(count):
                rows = pl.ds(pl.multiple_of((first + t) * SEG, SEG), SEG)
                for n, g in enumerate(range(0, G, WG)):
                    pltpu.make_async_copy(
                        buf.at[pl.ds(g, WG), rows], o_hbm.at[pl.ds(g, WG), rows],
                        wsem.at[0]).start(priority=n % 2)

        def compute(j, start_dmas):
            unit = _udiv(j, ncw, n_chunks)
            wi = j - unit * ncw
            cols = pl.ds(pl.multiple_of(wi * (CW // 2), CW // 2), CW // 2)
            rows = [pl.ds(pl.multiple_of((2 * unit + k) * W + wi * CW, CW), CW)
                    for k in range(2)]
            p = pbuf[slot_of(unit), :, cols, :].reshape(G * CW // 2, C)
            up = _repeat_rows(
                jnp.dot(p, wo[...], preferred_element_type=jnp.float32))
            c = jnp.concatenate(
                [buf[:, r, :].reshape(G * CW, C) for r in rows], axis=0)
            lat = jnp.dot(c, wc[...], preferred_element_type=jnp.float32)
            start_dmas()
            for k, r in enumerate(rows):
                o = lat[k * G * CW:(k + 1) * G * CW] + up
                buf[:, r, :] = o.astype(dtype).reshape(G, CW, C)

        wl_copy = pltpu.make_async_copy(wl_hbm, wl, ksem.at[0])
        wo_copy = pltpu.make_async_copy(wo_hbm, wo, ksem.at[1])
        wl_copy.start(priority=0)
        wo_copy.start(priority=1)
        lax.fori_loop(0, R_EARLY, lambda i, _: start_reads(i, 1), None)
        wl_copy.wait()
        wo_copy.wait()
        wc[...] = jnp.dot(
            wl[...], wo[...], preferred_element_type=jnp.float32).astype(dtype)
        lax.fori_loop(R_EARLY, R_BURST, lambda i, _: start_reads(i, 1), None)

        def read_phase(j, _):
            unit = _udiv(j, ncw, n_chunks)
            pl.when(j == unit * ncw)(lambda: wait_unit(unit))
            compute(j, lambda: start_reads(R_BURST + j * R_PER, R_PER))

        lax.fori_loop(0, n_read, read_phase, None)

        last = n_units - 1
        for unit in range(-(-n_read // ncw), last):
            wait_unit(unit)
        split = (n_steps - R_TAIL) * SEG
        wait_filled(buf.at[:, last * 2 * W:split], csem.at[slot_of(last)])
        lax.fori_loop(0, W_BURST // 2, lambda i, _: start_writes(2 * i, 2), None)
        wait_filled(buf.at[:, split:], csem.at[P_SLOTS])
        wait_filled(pbuf.at[slot_of(last)], psem.at[slot_of(last)])

        def write_phase(j, _):
            compute(j, lambda: start_writes(W_BURST + (j - n_read) * W_PER, W_PER))

        lax.fori_loop(n_read, n_chunks, write_phase, None)
        lax.fori_loop(n_steps - w_tail, n_steps,
                      lambda i, _: start_writes(i, 1), None)
        wait_filled(buf, wsem.at[0])

    out = pl.pallas_call(
        kernel,
        in_specs=[pl.BlockSpec(memory_space=pl.ANY)] * 4,
        out_specs=pl.BlockSpec(memory_space=pl.ANY),
        out_shape=jax.ShapeDtypeStruct((G, n_units * 2 * W, C), dtype),
        scratch_shapes=[
            pltpu.VMEM((G, n_units * 2 * W, C), dtype),
            pltpu.VMEM((P_SLOTS, G, W // 2, C), dtype),
            pltpu.VMEM((C, C), dtype),
            pltpu.VMEM((C, C), dtype),
            pltpu.VMEM((C, C), dtype),
            pltpu.SemaphoreType.DMA((P_SLOTS + 1,)),
            pltpu.SemaphoreType.DMA((P_SLOTS,)),
            pltpu.SemaphoreType.DMA((1,)),
            pltpu.SemaphoreType.DMA((2,)),
        ],
        compiler_params=pltpu.CompilerParams(
            vmem_limit_bytes=127 * 2**20,
            disable_bounds_checks=True,
            disable_semaphore_checks=True,
        ),
    )(
        c_fine.reshape(G, n_units * 2 * W, C),
        p_coarse.reshape(G, n_units, W // 2, C),
        w_lat,
        w_out.reshape(C, C),
    )
    return out.reshape(B, H, W, C)
```
